```python
import os as _os
_os.environ.setdefault("JAX_PLATFORMS", "cpu")
import jax
import jax.numpy as jnp

def _softmax(x, axis=-1):
    return jax.nn.softmax(x, axis=axis)
def _gelu(x):
    return jax.nn.gelu(x, approximate=True)
def _silu(x):
    return jax.nn.silu(x)
def _sigmoid(x):
    return jax.nn.sigmoid(x)
def _layernorm(x, axis=-1, eps=1e-5):
    m = jnp.mean(x, axis=axis, keepdims=True)
    v = jnp.var(x, axis=axis, keepdims=True)
    return (x - m) / jnp.sqrt(v + eps)
def _scatter_add(tgt, idx, src, axis=0):
    return tgt.at[idx].add(src)
def _segment_sum(src, seg, n):
    return jax.ops.segment_sum(src, seg, n)
class _Rng:
    def __init__(self, key):
        self._k = key
    def _next(self):
        self._k, sub = jax.random.split(self._k)
        return sub
    def normal(self, shape):
        return jax.random.normal(self._next(), shape, dtype=jnp.bfloat16)
    def randint(self, lo, hi, shape):
        return jax.random.randint(self._next(), shape, lo, hi, dtype=jnp.int32)
    def uniform(self, shape, lo=0.0, hi=1.0):
        return jax.random.uniform(self._next(), shape, jnp.bfloat16, lo, hi)
    def permutation(self, n):
        return jax.random.permutation(self._next(), n)


kernel_name = 'standalone__gqa_block_cached__near_ridge'

def setup_inputs():
    _rng = _Rng(jax.random.key(int.from_bytes(__import__("os").urandom(4), "little")))
    _w = (lambda a: (lambda t: t.astype(jnp.bfloat16) if jnp.issubdtype(t.dtype, jnp.floating) else t)(jnp.asarray(a)))
    B, Sq, D = 8, 80, 512
    Hq, Hkv, Sk, Dh = 32, 8, 2048, 128
    assert Hq % Hkv == 0, (Hq, Hkv)
    return {
        "x": _w((lambda *s: _rng.normal(s) * 0.8)(B, Sq, D)),
        "k_cache": _w((lambda *s: _rng.normal(s) * 0.8)(B, Hkv, Sk, Dh)),
        "v_cache": _w((lambda *s: _rng.normal(s) * 0.05)(B, Hkv, Sk, Dh)),
        "wq": _w((lambda *s: _rng.normal(s) * 0.8)(D, Hq * Dh) * (D ** -0.5)),
        "wo": _w((lambda *s: _rng.normal(s) * 0.05)(Hq * Dh, D) * ((Hq * Dh) ** -0.5)),
    }

def reference(x, k_cache, v_cache, wq, wo):
    B, Sq, D = x.shape
    Hq, Dh = 32, 128
    Hkv = k_cache.shape[1]
    rep = Hq // Hkv
    q = (lambda x, *d: x.transpose(*d))((x @ wq).reshape(B, Sq, Hq, Dh), 0, 2, 1, 3)
    k = jnp.repeat(k_cache, rep, axis=1)
    v = jnp.repeat(v_cache, rep, axis=1)
    scores = jnp.einsum("bhqd,bhkd->bhqk", q, k) * (Dh ** -0.5)
    p = _softmax(scores, axis=-1)
    o = jnp.einsum("bhqk,bhkd->bhqd", p, v)
    return (lambda x, *d: x.transpose(*d))(o, 0, 2, 1, 3).reshape(B, Sq, Hq * Dh) @ wo
```

```python
import math

import jax
import jax.experimental.pallas as pl
import jax.experimental.pallas.tpu as pltpu
import jax.numpy as jnp
from jax import lax

LANES = 128
KEY_CHUNK = 512
KV_SLOTS = 4
PRO_GROUPS = 2
OUT_START = 8


@jax.jit
def pallas_standalone__gqa_block_cached__near_ridge_kernel(
    x: jax.Array,
    k_cache: jax.Array,
    v_cache: jax.Array,
    wq: jax.Array,
    wo: jax.Array,
):
    B, Sq, D = x.shape
    _, Hkv, Sk, Dh = k_cache.shape
    rep = wq.shape[1] // Dh // Hkv
    W = rep * Dh
    T = B * Hkv
    n_chunks = Sk // KEY_CHUNK
    n_first = n_chunks // 2
    n_cols = D // LANES
    units = B * rep
    dtype = x.dtype
    f32 = jnp.float32
    assert dtype == jnp.bfloat16 and Dh == LANES and n_cols == rep and rep % 2 == 0
    assert Sq % 16 == 0 and Sk % (2 * KEY_CHUNK) == 0
    assert B & (B - 1) == 0 and B % KV_SLOTS == 0 and Hkv == B
    q_scale = (Dh**-0.5) * math.log2(math.e)

    q_sched = {v: [v] for v in range(units - PRO_GROUPS * rep)}
    o_sched = {}
    for v in range(units - rep):
        p = min(max(OUT_START + v, rep * (v // rep) + rep + 1), units - 1)
        o_sched.setdefault(p, []).append(v)
    x_parts = [(0, 1)]
    while x_parts[-1][0] + x_parts[-1][1] < B:
        done = x_parts[-1][0] + x_parts[-1][1]
        x_parts.append((done, done))

    sem_k, sem_v, sem_wq, sem_wo, sem_x = 0, KV_SLOTS, 2 * KV_SLOTS, 2 * KV_SLOTS + 1, 2 * KV_SLOTS + 2
    sem_w0 = sem_x + len(x_parts)
    sem_out = sem_x
    n_sems = sem_w0 + PRO_GROUPS

    def kernel(x_hbm, k_hbm, v_hbm, wq_hbm, wo_hbm, out_hbm,
               x_v, w0_v, x_s, kv_v, wq_v, wo_v, q_s, s_s, carry_s, o_s, acc_s, out_v, sems):
        def aligned(v, n):
            return v if isinstance(v, int) else pl.multiple_of(v, n)

        def k_copy(i, u):
            slot = u % KV_SLOTS
            return pltpu.make_async_copy(k_hbm.at[u % B, i + u // B], kv_v.at[slot], sems.at[sem_k + slot])

        def v_copy(i, u):
            slot = u % KV_SLOTS
            return pltpu.make_async_copy(
                v_hbm.at[u % B, i + u // B], kv_v.at[KV_SLOTS + slot], sems.at[sem_v + slot])

        def wq_copies(g):
            return [pltpu.make_async_copy(wq_hbm.at[:, pl.ds(aligned(g * W + h * Dh, Dh), Dh)],
                                          wq_v.at[g, h], sems.at[sem_wq]) for h in range(rep)]

        def wo_copies(g):
            return [pltpu.make_async_copy(wo_hbm.at[pl.ds(aligned(g * W, W), W), pl.ds(n * LANES, LANES)],
                                          wo_v.at[g, n], sems.at[sem_wo]) for n in range(n_cols)]

        def w0_copy(g):
            return pltpu.make_async_copy(
                wq_hbm.at[:, pl.ds(aligned(g * W, W), W)], w0_v.at[g], sems.at[sem_w0 + g])

        def x_copy(j):
            rows = pl.ds(x_parts[j][0] * Sq, x_parts[j][1] * Sq)
            return pltpu.make_async_copy(x_hbm.at[rows], x_v.at[rows], sems.at[sem_x + j])

        def out_copy(b):
            rows = pl.ds(b * Sq, Sq)
            return pltpu.make_async_copy(out_v.at[rows], out_hbm.at[rows], sems.at[sem_out])

        def start(copies):
            for cp in copies:
                cp.start()

        def wait(copies):
            for cp in copies:
                cp.wait()

        def load(ref, row0, rows):
            words = ref.bitcast(jnp.uint32)[pl.ds(row0 // 2, rows // 2), :]
            return pltpu.bitcast(words, dtype)

        def x_rows(b):
            return jnp.concatenate([load(x_s.at[b, j], 0, Sq) for j in range(n_cols)], axis=1)

        def split(t):
            if isinstance(t, int):
                return t // B, t % B
            return t >> (B.bit_length() - 1), t & (B - 1)

        def q_proj_group(g, b):
            for j in range(n_cols):
                x_s[b, j] = x_v[b * Sq:(b + 1) * Sq, j * LANES:(j + 1) * LANES]
            q = jnp.dot(x_rows(b), w0_v[g], preferred_element_type=f32)
            for h in range(rep):
                q_s[g * B + b, h] = (q[:, h * Dh:(h + 1) * Dh] * q_scale).astype(dtype)

        def q_proj(t, h):
            g, b = split(t)
            q = jnp.dot(x_rows(b), load(wq_v.at[g, h], 0, D), preferred_element_type=f32)
            q_s[t, h] = (q * q_scale).astype(dtype)

        def scores(t, h, slot, zero):
            q = load(q_s.at[t, h], 0, Sq)
            m = None
            for j in range(n_chunks):
                k = load(kv_v.at[slot], j * KEY_CHUNK, KEY_CHUNK)
                s = lax.dot_general(q, k, (((1,), (1,)), ((), ())), preferred_element_type=f32)
                s_s[h % 2 + zero, :, j * KEY_CHUNK:(j + 1) * KEY_CHUNK] = s
                for n in range(KEY_CHUNK // LANES):
                    sn = s[:, n * LANES:(n + 1) * LANES]
                    m = sn if m is None else jnp.maximum(m, sn)
            return jnp.max(m, axis=1, keepdims=True)

        def weigh(m, h, slot, zero, chunks, l, acc):
            if m.shape[1] != 1:
                m = jnp.concatenate([m] * (KEY_CHUNK // LANES), axis=1)
            for j in chunks:
                v = load(kv_v.at[KV_SLOTS + slot], j * KEY_CHUNK, KEY_CHUNK)
                p = jnp.exp2(s_s[h % 2 + zero, :, j * KEY_CHUNK:(j + 1) * KEY_CHUNK] - m)
                lj = None
                for n in range(KEY_CHUNK // LANES):
                    pn = p[:, n * LANES:(n + 1) * LANES]
                    lj = pn if lj is None else lj + pn
                l = lj if l is None else l + lj
                r = jnp.dot(p.astype(dtype), v, preferred_element_type=f32)
                acc = r if acc is None else acc + r
            return l, acc

        def finish(l, acc, t, h):
            l = jnp.sum(l, axis=1, keepdims=True)
            r = pl.reciprocal(l, approx=True)
            r = r * (2.0 - l * r)
            o_s[t + 1, h] = (acc * r).astype(dtype)

        def out_proj(t, n, last):
            g, b = split(t)
            o = jnp.concatenate([load(o_s.at[t + 1, h], 0, Sq) for h in range(rep)], axis=1)
            r = jnp.dot(o, load(wo_v.at[g, n], 0, W), preferred_element_type=f32)
            rows = pl.ds(aligned(b * Sq, Sq), Sq)
            cols = slice(n * LANES, (n + 1) * LANES)
            total = acc_s[rows, cols] + r
            if last:
                out_v[rows, cols] = total.astype(dtype)
            else:
                acc_s[rows, cols] = total

        def if_step_exists(i, u, fn):
            if u < B:
                fn()
            else:
                pl.when(i + u // B < Hkv)(fn)

        def after_last_k_use(i, u):
            if_step_exists(i, u + KV_SLOTS, lambda: k_copy(i, u + KV_SLOTS).start())
            g_next = i + PRO_GROUPS + 1
            if u == 0:
                pl.when(g_next < Hkv)(lambda: start(wq_copies(g_next)))
            if u == (OUT_START - rep) // rep:
                wait(wo_copies(i))
                pl.when(i + 1 < Hkv)(lambda: start(wo_copies(i + 1)))
            if u == B - 1:
                pl.when(g_next < Hkv)(lambda: wait(wq_copies(g_next)))

        def before_first_v_use(i, u):
            if_step_exists(i, u - 1 + KV_SLOTS, lambda: v_copy(i, u - 1 + KV_SLOTS).start())
            v_copy(i, u).wait()

        x_copy(0).start()
        w0_copy(0).start()
        for j in range(1, len(x_parts)):
            x_copy(j).start()
        for g in range(1, PRO_GROUPS):
            w0_copy(g).start()
        k_copy(0, 0).start()
        v_copy(0, 0).start()
        start(wq_copies(PRO_GROUPS))
        for u in range(1, KV_SLOTS):
            k_copy(0, u).start()
            if u < KV_SLOTS - 1:
                v_copy(0, u).start()
            if u == min(KV_SLOTS - 1, OUT_START // rep):
                start(wo_copies(0))
        acc_s[...] = jnp.zeros_like(acc_s)
        carry_s[...] = jnp.ones_like(carry_s)
        s_s[1] = jnp.zeros((Sq, Sk), f32)
        kv_v[2 * KV_SLOTS - 1] = jnp.zeros((Sk, Dh), dtype)

        def first_groups(g, _):
            for j, (b0, nb) in enumerate(x_parts):
                pl.when(g == 0)(x_copy(j).wait)
                if j == 0:
                    w0_copy(g).wait()
                for b in range(b0, b0 + nb):
                    q_proj_group(g, b)
            return 0

        lax.fori_loop(0, PRO_GROUPS, first_groups, 0)
        wait(wq_copies(PRO_GROUPS))

        def group(i, _):
            zero = (i * (i + 1)) & 1
            m, l, acc = carry_s[0], carry_s[1], carry_s[2]
            for p in range(units):
                u, h = divmod(p, rep)
                u_prev, h_prev = divmod(p - 1, rep)
                if h == 0:
                    k_copy(i, u).wait()
                m_next = scores(i * B + u, h, u % KV_SLOTS, zero)
                if h == rep - 1:
                    after_last_k_use(i, u)
                for v in o_sched.get(p, []):
                    out_proj((B - 1) * i + v // rep, v % rep, False)
                l, acc = weigh(m, h_prev, u_prev % KV_SLOTS, zero, range(n_first, n_chunks), l, acc)
                if h == 0:
                    before_first_v_use(i, u)
                finish(l, acc, i * B + u_prev, h_prev)
                for v in q_sched.get(p, []):
                    q_proj(PRO_GROUPS * B + (B - PRO_GROUPS) * i + v // rep, v % rep)
                l, acc = weigh(m_next, h, u % KV_SLOTS, zero, range(n_first), None, None)
                m = m_next
            carry_s[0] = jnp.broadcast_to(m, (Sq, LANES))
            carry_s[1] = l
            carry_s[2] = acc
            return 0

        lax.fori_loop(0, Hkv, group, 0)

        l, acc = weigh(carry_s[0], rep - 1, (B - 1) % KV_SLOTS, 0, range(n_first, n_chunks),
                       carry_s[1], carry_s[2])
        finish(l, acc, T - 1, rep - 1)
        for b in range(B):
            for n in range(n_cols):
                out_proj(T - B + b, n, True)
            out_copy(b).start()
        for b in range(B):
            out_copy(b).wait()

    hbm = pl.BlockSpec(memory_space=pl.ANY)
    out = pl.pallas_call(
        kernel,
        in_specs=[hbm] * 5,
        out_specs=hbm,
        out_shape=jax.ShapeDtypeStruct((B * Sq, D), dtype),
        scratch_shapes=[
            pltpu.VMEM((B * Sq, D), dtype),
            pltpu.VMEM((PRO_GROUPS, D, W), dtype),
            pltpu.VMEM((B, n_cols, Sq, LANES), dtype),
            pltpu.VMEM((2 * KV_SLOTS, Sk, Dh), dtype),
            pltpu.VMEM((Hkv, rep, D, Dh), dtype),
            pltpu.VMEM((Hkv, n_cols, W, LANES), dtype),
            pltpu.VMEM((T, rep, Sq, Dh), dtype),
            pltpu.VMEM((2, Sq, Sk), f32),
            pltpu.VMEM((3, Sq, LANES), f32),
            pltpu.VMEM((T + 1, rep, Sq, Dh), dtype),
            pltpu.VMEM((B * Sq, D), f32),
            pltpu.VMEM((B * Sq, D), dtype),
            pltpu.SemaphoreType.DMA((n_sems,)),
        ],
        compiler_params=pltpu.CompilerParams(
            vmem_limit_bytes=64 * 1024 * 1024,
            disable_bounds_checks=True,
            flags={"XLA_TPU_RESCHEDULE_DMA_DONES": True},
        ),
    )(x.reshape(B * Sq, D), k_cache, v_cache, wq, wo)
    return out.reshape(B, Sq, D)
```

```python
import math

import jax
import jax.experimental.pallas as pl
import jax.experimental.pallas.tpu as pltpu
import jax.numpy as jnp
from jax import lax

LANES = 128
KEY_CHUNK = 512
KV_SLOTS = 4
PRO_GROUPS = 2
OUT_START = 8


@jax.jit
def pallas_standalone__gqa_block_cached__near_ridge_kernel(
    x: jax.Array,
    k_cache: jax.Array,
    v_cache: jax.Array,
    wq: jax.Array,
    wo: jax.Array,
):
    B, Sq, D = x.shape
    _, Hkv, Sk, Dh = k_cache.shape
    rep = wq.shape[1] // Dh // Hkv
    W = rep * Dh
    T = B * Hkv
    n_chunks = Sk // KEY_CHUNK
    n_first = n_chunks // 2
    n_cols = D // LANES
    units = B * rep
    dtype = x.dtype
    f32 = jnp.float32
    assert dtype == jnp.bfloat16 and Dh == LANES and n_cols == rep and rep % 2 == 0
    assert Sq % 16 == 0 and Sk % (2 * KEY_CHUNK) == 0
    assert B & (B - 1) == 0 and B % KV_SLOTS == 0 and Hkv == B
    q_scale = (Dh**-0.5) * math.log2(math.e)

    q_sched = {v - 1: [v] for v in range(1, units - PRO_GROUPS * rep)}
    o_sched = {}
    for v in range(units - rep):
        p = min(max(OUT_START + v, rep * (v // rep) + rep + 1), units - 1)
        o_sched.setdefault(p, []).append(v)
    x_parts = [(0, 1)]
    while x_parts[-1][0] + x_parts[-1][1] < B:
        done = x_parts[-1][0] + x_parts[-1][1]
        x_parts.append((done, done))

    sem_k, sem_v, sem_wq, sem_wo, sem_x = 0, KV_SLOTS, 2 * KV_SLOTS, 2 * KV_SLOTS + 1, 2 * KV_SLOTS + 2
    sem_w0 = sem_x + len(x_parts)
    sem_out = sem_x
    n_sems = sem_w0 + PRO_GROUPS

    def kernel(x_hbm, k_hbm, v_hbm, wq_hbm, wo_hbm, out_hbm,
               x_v, w0_v, x_s, kv_v, wq_v, wo_v, q_s, s_s, carry_s, o_s, acc_s, out_v, sems):
        def aligned(v, n):
            return v if isinstance(v, int) else pl.multiple_of(v, n)

        def k_copy(i, u):
            slot = u % KV_SLOTS
            return pltpu.make_async_copy(k_hbm.at[u % B, i + u // B], kv_v.at[slot], sems.at[sem_k + slot])

        def v_copy(i, u):
            slot = u % KV_SLOTS
            return pltpu.make_async_copy(
                v_hbm.at[u % B, i + u // B], kv_v.at[KV_SLOTS + slot], sems.at[sem_v + slot])

        def wq_copies(g):
            return [pltpu.make_async_copy(wq_hbm.at[:, pl.ds(aligned(g * W + h * Dh, Dh), Dh)],
                                          wq_v.at[g, h], sems.at[sem_wq]) for h in range(rep)]

        def wo_copies(g):
            return [pltpu.make_async_copy(wo_hbm.at[pl.ds(aligned(g * W, W), W), pl.ds(n * LANES, LANES)],
                                          wo_v.at[g, n], sems.at[sem_wo]) for n in range(n_cols)]

        def w0_copy(g):
            return pltpu.make_async_copy(
                wq_hbm.at[:, pl.ds(aligned(g * W, W), W)], w0_v.at[g], sems.at[sem_w0 + g])

        def x_copy(j):
            rows = pl.ds(x_parts[j][0] * Sq, x_parts[j][1] * Sq)
            return pltpu.make_async_copy(x_hbm.at[rows], x_v.at[rows], sems.at[sem_x + j])

        def out_copy(b):
            rows = pl.ds(b * Sq, Sq)
            return pltpu.make_async_copy(out_v.at[rows], out_hbm.at[rows], sems.at[sem_out])

        def start(copies):
            for cp in copies:
                cp.start()

        def wait(copies):
            for cp in copies:
                cp.wait()

        def load(ref, row0, rows):
            words = ref.bitcast(jnp.uint32)[pl.ds(row0 // 2, rows // 2), :]
            return pltpu.bitcast(words, dtype)

        def x_rows(b):
            return jnp.concatenate([load(x_s.at[b, j], 0, Sq) for j in range(n_cols)], axis=1)

        def split(t):
            if isinstance(t, int):
                return t // B, t % B
            return t >> (B.bit_length() - 1), t & (B - 1)

        def q_proj_group(g, b):
            for j in range(n_cols):
                x_s[b, j] = x_v[b * Sq:(b + 1) * Sq, j * LANES:(j + 1) * LANES]
            q = jnp.dot(x_rows(b), w0_v[g], preferred_element_type=f32)
            for h in range(rep):
                q_s[g * B + b, h] = (q[:, h * Dh:(h + 1) * Dh] * q_scale).astype(dtype)

        def q_proj(t, h):
            g, b = split(t)
            q = jnp.dot(x_rows(b), load(wq_v.at[g, h], 0, D), preferred_element_type=f32)
            q_s[t, h] = (q * q_scale).astype(dtype)

        def scores(t, h, slot, zero, before=None):
            q = load(q_s.at[t, h], 0, Sq)
            if before is not None:
                before()
            m = None
            for j in range(n_chunks):
                k = load(kv_v.at[slot], j * KEY_CHUNK, KEY_CHUNK)
                s = lax.dot_general(q, k, (((1,), (1,)), ((), ())), preferred_element_type=f32)
                s_s[h % 2 + zero, :, j * KEY_CHUNK:(j + 1) * KEY_CHUNK] = s
                for n in range(KEY_CHUNK // LANES):
                    sn = s[:, n * LANES:(n + 1) * LANES]
                    m = sn if m is None else jnp.maximum(m, sn)
            return jnp.max(m, axis=1, keepdims=True)

        def weigh(m, h, slot, zero, chunks, l, acc):
            if m.shape[1] != 1:
                m = jnp.concatenate([m] * (KEY_CHUNK // LANES), axis=1)
            for j in chunks:
                v = load(kv_v.at[KV_SLOTS + slot], j * KEY_CHUNK, KEY_CHUNK)
                p = jnp.exp2(s_s[h % 2 + zero, :, j * KEY_CHUNK:(j + 1) * KEY_CHUNK] - m)
                lj = None
                for n in range(KEY_CHUNK // LANES):
                    pn = p[:, n * LANES:(n + 1) * LANES]
                    lj = pn if lj is None else lj + pn
                l = lj if l is None else l + lj
                r = jnp.dot(p.astype(dtype), v, preferred_element_type=f32)
                acc = r if acc is None else acc + r
            return l, acc

        def finish(l, acc, t, h):
            l = jnp.sum(l, axis=1, keepdims=True)
            r = pl.reciprocal(l, approx=True)
            r = r * (2.0 - l * r)
            o_s[t + 1, h] = (acc * r).astype(dtype)

        def out_proj(t, n, last):
            g, b = split(t)
            o = jnp.concatenate([load(o_s.at[t + 1, h], 0, Sq) for h in range(rep)], axis=1)
            r = jnp.dot(o, load(wo_v.at[g, n], 0, W), preferred_element_type=f32)
            rows = pl.ds(aligned(b * Sq, Sq), Sq)
            cols = slice(n * LANES, (n + 1) * LANES)
            total = acc_s[rows, cols] + r
            if last:
                out_v[rows, cols] = total.astype(dtype)
            else:
                acc_s[rows, cols] = total

        def if_step_exists(i, u, fn):
            if u < B:
                fn()
            else:
                pl.when(i + u // B < Hkv)(fn)

        def after_last_k_use(i, u):
            if_step_exists(i, u + KV_SLOTS, lambda: k_copy(i, u + KV_SLOTS).start())
            g_next = i + PRO_GROUPS + 1
            if u == 0:
                pl.when(g_next < Hkv)(lambda: start(wq_copies(g_next)))
            if u == (OUT_START - rep) // rep:
                wait(wo_copies(i))
                pl.when(i + 1 < Hkv)(lambda: start(wo_copies(i + 1)))
            if u == B - 1:
                pl.when(g_next < Hkv)(lambda: wait(wq_copies(g_next)))

        def before_first_v_use(i, u):
            if_step_exists(i, u - 1 + KV_SLOTS, lambda: v_copy(i, u - 1 + KV_SLOTS).start())
            v_copy(i, u).wait()

        x_copy(0).start()
        w0_copy(0).start()
        for j in range(1, len(x_parts)):
            x_copy(j).start()
        for g in range(1, PRO_GROUPS):
            w0_copy(g).start()
        k_copy(0, 0).start()
        v_copy(0, 0).start()
        start(wq_copies(PRO_GROUPS))
        for u in range(1, KV_SLOTS):
            k_copy(0, u).start()
            if u < KV_SLOTS - 1:
                v_copy(0, u).start()
            if u == min(KV_SLOTS - 1, OUT_START // rep):
                start(wo_copies(0))
        acc_s[...] = jnp.zeros_like(acc_s)
        carry_s[...] = jnp.ones_like(carry_s)
        s_s[1] = jnp.zeros((Sq, Sk), f32)
        kv_v[2 * KV_SLOTS - 1] = jnp.zeros((Sk, Dh), dtype)

        def first_groups(g, _):
            for j, (b0, nb) in enumerate(x_parts):
                pl.when(g == 0)(x_copy(j).wait)
                if j == 0:
                    w0_copy(g).wait()
                for b in range(b0, b0 + nb):
                    q_proj_group(g, b)
            return 0

        lax.fori_loop(0, PRO_GROUPS, first_groups, 0)
        wait(wq_copies(PRO_GROUPS))

        def group(i, _):
            zero = (i * (i + 1)) & 1
            q_base = PRO_GROUPS * B + (B - PRO_GROUPS) * i
            m, l, acc = carry_s[0], carry_s[1], carry_s[2]
            for p in range(units):
                u, h = divmod(p, rep)
                u_prev, h_prev = divmod(p - 1, rep)
                if h == 0:
                    k_copy(i, u).wait()
                m_next = scores(i * B + u, h, u % KV_SLOTS, zero,
                                (lambda: q_proj(q_base, 0)) if p == 0 else None)
                if h == rep - 1:
                    after_last_k_use(i, u)
                for v in o_sched.get(p, []):
                    out_proj((B - 1) * i + v // rep, v % rep, False)
                l, acc = weigh(m, h_prev, u_prev % KV_SLOTS, zero, range(n_first, n_chunks), l, acc)
                if h == 0:
                    before_first_v_use(i, u)
                finish(l, acc, i * B + u_prev, h_prev)
                for v in q_sched.get(p, []):
                    q_proj(q_base + v // rep, v % rep)
                l, acc = weigh(m_next, h, u % KV_SLOTS, zero, range(n_first), None, None)
                m = m_next
            carry_s[0] = jnp.broadcast_to(m, (Sq, LANES))
            carry_s[1] = l
            carry_s[2] = acc
            return 0

        lax.fori_loop(0, Hkv, group, 0)

        l, acc = weigh(carry_s[0], rep - 1, (B - 1) % KV_SLOTS, 0, range(n_first, n_chunks),
                       carry_s[1], carry_s[2])
        finish(l, acc, T - 1, rep - 1)
        for b in range(B):
            for n in range(n_cols):
                out_proj(T - B + b, n, True)
            out_copy(b).start()
        for b in range(B):
            out_copy(b).wait()

    hbm = pl.BlockSpec(memory_space=pl.ANY)
    out = pl.pallas_call(
        kernel,
        in_specs=[hbm] * 5,
        out_specs=hbm,
        out_shape=jax.ShapeDtypeStruct((B * Sq, D), dtype),
        scratch_shapes=[
            pltpu.VMEM((B * Sq, D), dtype),
            pltpu.VMEM((PRO_GROUPS, D, W), dtype),
            pltpu.VMEM((B, n_cols, Sq, LANES), dtype),
            pltpu.VMEM((2 * KV_SLOTS, Sk, Dh), dtype),
            pltpu.VMEM((Hkv, rep, D, Dh), dtype),
            pltpu.VMEM((Hkv, n_cols, W, LANES), dtype),
            pltpu.VMEM((T, rep, Sq, Dh), dtype),
            pltpu.VMEM((2, Sq, Sk), f32),
            pltpu.VMEM((3, Sq, LANES), f32),
            pltpu.VMEM((T + 1, rep, Sq, Dh), dtype),
            pltpu.VMEM((B * Sq, D), f32),
            pltpu.VMEM((B * Sq, D), dtype),
            pltpu.SemaphoreType.DMA((n_sems,)),
        ],
        compiler_params=pltpu.CompilerParams(
            vmem_limit_bytes=64 * 1024 * 1024,
            disable_bounds_checks=True,
            flags={"XLA_TPU_RESCHEDULE_DMA_DONES": True},
        ),
    )(x.reshape(B * Sq, D), k_cache, v_cache, wq, wo)
    return out.reshape(B, Sq, D)
```
